```python
import jax
import jax.numpy as jnp

def _softmax(x, axis=-1):
    return jax.nn.softmax(x, axis=axis)

def _gelu(x):
    return jax.nn.gelu(x, approximate=True)

def _silu(x):
    return jax.nn.silu(x)

def _sigmoid(x):
    return jax.nn.sigmoid(x)

def _layernorm(x, axis=-1, eps=1e-05):
    m = jnp.mean(x, axis=axis, keepdims=True)
    v = jnp.var(x, axis=axis, keepdims=True)
    return (x - m) / jnp.sqrt(v + eps)

def _scatter_add(tgt, idx, src, axis=0):
    return tgt.at[idx].add(src)

def _segment_sum(src, seg, n):
    return jax.ops.segment_sum(src, seg, n)

class _Rng:

    def __init__(self, key):
        self._k = key

    def _next(self):
        self._k, sub = jax.random.split(self._k)
        return sub

    def normal(self, shape):
        return jax.random.normal(self._next(), shape, dtype=jnp.bfloat16)

    def randint(self, lo, hi, shape):
        return jax.random.randint(self._next(), shape, lo, hi, dtype=jnp.int32)

    def uniform(self, shape, lo=0.0, hi=1.0):
        return jax.random.uniform(self._next(), shape, jnp.bfloat16, lo, hi)

    def permutation(self, n):
        return jax.random.permutation(self._next(), n)
kernel_name = 'adaLN_cond__grouped_kv_mqa__dense_activation_silu__prompt'

def _fwd_setup_inputs():
    _rng = _Rng(jax.random.key(int.from_bytes(__import__("os").urandom(4), "little")))
    _w = lambda a: (lambda t: t.astype(jnp.bfloat16) if jnp.issubdtype(t.dtype, jnp.floating) else t)(jnp.asarray(a))

    def _A_setup():
        B, S, D, H = (1, 2048, 640, 32)
        Dh = D // H
        return {'x': _w((lambda *s: _rng.normal(s) * 0.05)(B, S, D)), 'wq': _w((lambda *s: _rng.normal(s) * 0.05)(D, H * Dh)), 'wk': _w((lambda *s: _rng.normal(s) * 0.05)(D, Dh)), 'wv': _w((lambda *s: _rng.normal(s) * 0.05)(D, Dh)), 'wo': _w((lambda *s: _rng.normal(s) * 0.05)(H * Dh, D))}
    _A_in = _A_setup()

    def _B_setup():
        B, S, D, F = (1, 2048, 640, 1728)
        return {'x': _w((lambda *s: _rng.normal(s) * 0.05)(B, S, D)), 'w1': _w((lambda *s: _rng.normal(s) * 0.05)(D, F) * D ** (-0.5)), 'w2': _w((lambda *s: _rng.normal(s) * 0.05)(F, D) * F ** (-0.5))}
    _B_in = _B_setup()
    return {'A_x': _A_in['x'], 'A_wq': _A_in['wq'], 'A_wk': _A_in['wk'], 'A_wv': _A_in['wv'], 'A_wo': _A_in['wo'], 'B_x': _B_in['x'], 'B_w1': _B_in['w1'], 'B_w2': _B_in['w2'], 'c': _w((lambda *s: _rng.normal(s) * 0.05)(1, 640)), 'w_mod': _w((lambda *s: _rng.normal(s) * 0.05)(640, 6 * 640) * 640 ** (-0.5))}

def _fwd_reference(A_x, A_wq, A_wk, A_wv, A_wo, B_x, B_w1, B_w2, c, w_mod):

    def _A_ref(x, wq, wk, wv, wo):
        B, S, D = x.shape
        H = 32
        Dh = D // H
        q = (lambda x, *d: x.transpose(*d))((x @ wq).reshape(B, S, H, Dh), 0, 2, 1, 3)
        k = x @ wk
        v = x @ wv
        scores = jnp.einsum('bhqd,bkd->bhqk', q, k) * Dh ** (-0.5)
        p = _softmax(scores, axis=-1)
        o = jnp.einsum('bhqk,bkd->bhqd', p, v)
        return (lambda x, *d: x.transpose(*d))(o, 0, 2, 1, 3).reshape(B, S, H * Dh) @ wo

    def _B_ref(x, w1, w2):
        h = jnp.einsum('bsd,df->bsf', x, w1)
        h = _silu(h)
        out = jnp.einsum('bsf,fd->bsd', h, w2)
        return out
    x = A_x
    mod = (_silu(c) @ w_mod).reshape(c.shape[0], 6, 1, -1)
    sa, ca, ga, sb, cb, gb = (mod[:, 0].copy(), mod[:, 1].copy(), mod[:, 2].copy(), mod[:, 3].copy(), mod[:, 4].copy(), mod[:, 5].copy())
    h = _layernorm(x, axis=-1) * (1 + ca) + sa
    x = x + ga * _A_ref(h, A_wq, A_wk, A_wv, A_wo)
    h = _layernorm(x, axis=-1) * (1 + cb) + sb
    x = x + gb * _B_ref(h, B_w1, B_w2)
    return x

def setup_inputs():
    _inp = _fwd_setup_inputs()
    _gk = jax.random.fold_in(jax.random.key(int.from_bytes(__import__("os").urandom(4), "little")), 2 ** 31 - 1)
    _shapes = [[1, 2048, 640]]
    _dtypes = ['bfloat16']
    _gks = jax.random.split(_gk, len(_shapes))
    _gs = [jax.random.normal(k, s, dtype=jnp.dtype(d)) * 0.05 for k, s, d in zip(_gks, _shapes, _dtypes)]
    _inp['grad_out'] = _gs[0]
    return _inp

def reference(A_x, A_wq, A_wk, A_wv, A_wo, B_w1, B_w2, c, w_mod, B_x, grad_out):
    _const = dict(B_x=B_x)

    def _f(*_d):
        return _fwd_reference(**{'A_x': _d[0], 'A_wq': _d[1], 'A_wk': _d[2], 'A_wv': _d[3], 'A_wo': _d[4], 'B_w1': _d[5], 'B_w2': _d[6], 'c': _d[7], 'w_mod': _d[8], **_const})
    _out, _vjp = jax.vjp(_f, A_x, A_wq, A_wk, A_wv, A_wo, B_w1, B_w2, c, w_mod)
    _grads = _vjp(grad_out)
    _out0 = jnp.asarray(_out)
    return (_out0, *[jnp.asarray(_g) for _g in _grads])
```

```python
import math

import jax
import jax.numpy as jnp
from jax import lax
import jax.experimental.pallas as pl
import jax.experimental.pallas.tpu as pltpu

S, D, H, F = 2048, 640, 32, 1728
DH = D // H
HR = 24
W = 512
NB = S // W
C = 128
NC = S // C
FC = 432
BWD_UNROLL = 2
EPS = 1e-5
LOG2E = math.log2(math.e)
SCALE = DH ** -0.5

bf16, f32, u32 = jnp.bfloat16, jnp.float32, jnp.uint32
NN = (((1,), (0,)), ((), ()))
NT = (((1,), (1,)), ((), ()))


def _dot(a, b, dims=NN):
    return lax.dot_general(a, b, dims, preferred_element_type=f32)


def _pack(x):
    return pltpu.bitcast(x, u32)


def _unpack(x):
    return pltpu.bitcast(x, bf16)


def _round(x):
    return x.astype(bf16).astype(f32)


def _lanes(col, n):
    return jnp.concatenate([col] * (n // 128), axis=1)


def _fold(x):
    out = x[:, :128]
    for i in range(1, x.shape[1] // 128):
        out = out + x[:, i * 128:(i + 1) * 128]
    return out


def _column(row):
    return jnp.broadcast_to(row, (128, D)).T


def _layernorm(x):
    xc = x - jnp.sum(x, axis=0, keepdims=True) * (1.0 / D)
    rstd = lax.rsqrt(jnp.sum(xc * xc, axis=0, keepdims=True) * (1.0 / D) + EPS)
    return xc * rstd, rstd


def _layernorm_bwd(dxhat, xhat, rstd):
    m1 = jnp.sum(dxhat, axis=0, keepdims=True) * (1.0 / D)
    m2 = jnp.sum(dxhat * xhat, axis=0, keepdims=True) * (1.0 / D)
    return (dxhat - m1 - xhat * m2) * rstd


def _to_heads(x):
    out = []
    for j in range(H // 2):
        r = 2 * DH * j
        out.append(x[r:r + HR])
        out.append(pltpu.roll(x[r + 16:r + 16 + HR], DH, 0))
    return out


def _from_heads(heads):
    low = lax.broadcasted_iota(jnp.int32, (8, W), 0) < 4
    rows = []
    for j in range(H // 2):
        even, odd = heads[2 * j], pltpu.roll(heads[2 * j + 1], HR - DH, 0)
        rows += [even[:16], jnp.where(low, even[16:], odd[:8]), odd[8:]]
    return jnp.concatenate(rows, axis=0)


def _as_weights(x):
    return jnp.concatenate([x, jnp.zeros((32 - HR, W), f32)], axis=0).astype(bf16)


def _kernel(c_ref, wkT_ref, wvT_ref, x_hbm, g_hbm, wq_hbm, wo_hbm, w1T_hbm, w2_hbm, wmod_hbm,
            out_hbm, dx_hbm, dwq_hbm, dwkT_ref, dwvT_ref, dwo_hbm, dw1T_hbm, dw2_hbm, dc_ref,
            dwmod_hbm,
            xT, QH, OH, KS, VS, KT, VT, DK, DV, wq, wo, woT, w1T, w1, w2, w2T, wkv,
            dw1, dw2, dwo, dx1T, mod, dmod, gbuf, obuf, SA, MA, in_sem, g_sem, o_sem, out_sem):
    SA_, CA_, GA_, SB_, CB_, GB_ = range(6)

    def g_copy(b):
        return pltpu.make_async_copy(g_hbm.at[pl.ds(b * W, W)], gbuf, g_sem)

    def o_copy(b):
        return pltpu.make_async_copy(obuf, out_hbm.at[pl.ds(b * W, W)], o_sem)

    def rows(c):
        return slice(c * C // 2, (c + 1) * C // 2)

    def scores(c, q):
        return _dot(_unpack(KS[rows(c), :])[:, :32], q)

    def colmax(s):
        return jnp.max(s.reshape(C // 8, 8, W), axis=0)

    def finish_max(m):
        return jnp.broadcast_to(jnp.max(m, axis=0, keepdims=True), (8, W))

    cf = c_ref[...].astype(f32)
    sig_c = jax.nn.sigmoid(cf)
    silu_c = _round(cf * sig_c)

    def prologue(xbuf, wqT, wmod):
        lo, hi = pl.ds(0, 2 * D), pl.ds(2 * D, 4 * D)
        srcs = [(wmod_hbm.at[:, lo], wmod.at[:, lo]), (wq_hbm, wq)]
        srcs += [(x_hbm.at[pl.ds(b * W, W)], xbuf.at[b]) for b in range(NB)]
        srcs += [(wo_hbm, wo), (w1T_hbm, w1T), (w2_hbm, w2), (wmod_hbm.at[:, hi], wmod.at[:, hi])]
        copies = [pltpu.make_async_copy(s, d, in_sem.at[i]) for i, (s, d) in enumerate(srcs)]
        for cp in copies:
            cp.start()
        g_copy(0).start()

        for ref in (wkv, DK, DV, dw1, dw2, dwo, dmod):
            ref[...] = jnp.zeros(ref.shape, f32)
        wkv[0:DH, :] = wkT_ref[...].astype(f32)
        wkv[HR:HR + DH, :] = wvT_ref[...].astype(f32)

        def modulation(k):
            row = _dot(jnp.broadcast_to(silu_c, (8, D)), wmod[:, k * D:(k + 1) * D])[0:1]
            mod[k] = _column(row + 1.0 if k in (CA_, CB_) else row)

        copies[0].wait()
        modulation(SA_)
        modulation(CA_)
        copies[1].wait()
        wqT[...] = wq[...].T
        row = lax.broadcasted_iota(jnp.int32, (HR, W), 0)
        pad = jnp.zeros((128 - HR, W), f32)
        for b in range(NB):
            copies[2 + b].wait()
            xt = xbuf[b].T
            xT[b] = _pack(xt)
            xhat, _ = _layernorm(xt.astype(f32))
            h = (xhat * _lanes(mod[CA_], W) + _lanes(mod[SA_], W)).astype(bf16)
            kv = _round(_dot(wkv[0:2 * HR, :], h))
            k = kv[:HR]
            v = jnp.where(jnp.logical_and(row >= DH, row < DH + 3), 1.0, kv[HR:])
            KT[:, b * W:(b + 1) * W] = k
            VT[:, b * W:(b + 1) * W] = v
            KS[b * W // 2:(b + 1) * W // 2, :] = _pack(jnp.concatenate([k, pad], 0).T.astype(bf16))
            VS[b * W // 2:(b + 1) * W // 2, :] = _pack(jnp.concatenate([v, pad], 0).T.astype(bf16))
            q = _round(_dot(wqT[...], h) * (SCALE * LOG2E))
            for i, win in enumerate(_to_heads(q)):
                QH[b * H + i] = win
        for cp in copies[2 + NB:]:
            cp.wait()
        woT[...] = wo[...].T
        w1[...] = w1T[...].T
        w2T[...] = w2[...].T
        for k in (GA_, SB_, CB_, GB_):
            modulation(k)
        q = _as_weights(QH[0])
        m = None
        for c in range(NC):
            s = scores(c, q)
            SA[c * C:(c + 1) * C, :] = s
            m = colmax(s) if m is None else jnp.maximum(m, colmax(s))
        MA[...] = finish_max(m)

    pl.run_scoped(prologue, pltpu.VMEM((NB, W, D), bf16), pltpu.VMEM((D, D), bf16),
                  pltpu.VMEM((D, 6 * D), bf16))

    def attention_fwd(b, P, SB, MB):
        def head(h, s_cur, m_cur, s_nxt, m_nxt):
            q = _as_weights(QH[jnp.minimum(b * H + h + 1, NB * H - 1)])
            mx = m_cur[...]
            m = o = p = None
            for c in range(NC + 1):
                prev = p
                if c < NC:
                    s = scores(c, q)
                    s_nxt[c * C:(c + 1) * C, :] = s
                    m = colmax(s) if m is None else jnp.maximum(m, colmax(s))
                    t = s_cur[c * C:(c + 1) * C, :].reshape(C // 8, 8, W) - mx[None]
                    p = jnp.exp2(t.reshape(C, W)).astype(bf16)
                    P[h, rows(c), :] = _pack(p)
                if c > 0:
                    part = _dot(VT[:, (c - 1) * C:c * C], prev)
                    o = part if o is None else o + part
            m_nxt[...] = finish_max(m)
            OH[h] = o

        def body(j, carry):
            head(2 * j, SA, MA, SB, MB)
            head(2 * j + 1, SB, MB, SA, MA)
            return carry

        lax.fori_loop(0, H // 2, body, 0)

    def dense(b, aT, duT):
        def normalized(i):
            raw = OH[i]
            inv_l = 1.0 / raw[DH:DH + 1]
            return raw * inv_l, inv_l

        g_copy(b).wait()
        oT = _from_heads([normalized(i)[0] for i in range(H)]).astype(bf16)
        attn = _dot(woT[...], oT)

        gT = gbuf[...].T
        ga, gb, cb = _lanes(mod[GA_], W), _lanes(mod[GB_], W), _lanes(mod[CB_], W)
        dm = (gT.astype(f32) * gb).astype(bf16)
        x1 = _unpack(xT[b]).astype(f32) + ga * attn
        dx1T[b] = x1
        xhat, rstd = _layernorm(x1)
        h2 = (xhat * cb + _lanes(mod[SB_], W)).astype(bf16)
        chunks = [slice(i * FC, (i + 1) * FC) for i in range(F // FC)]
        for sl in chunks:
            da = _dot(w2[sl, :], dm)
            u = _dot(w1T[sl, :], h2)
            sig = jax.nn.sigmoid(u)
            a = u * sig
            aT[sl, :] = a.astype(bf16)
            duT[sl, :] = (da * (sig + a * (1.0 - sig))).astype(bf16)
        mlp = _dot(w2T[...], aT[...])
        dmod[GB_] += _fold(gT.astype(f32) * mlp)
        obuf[...] = (dx1T[b] + gb * mlp).astype(bf16).T

        dh2 = _dot(w1[...], duT[...])
        for sl in chunks:
            dw2[sl, :] += _dot(aT[sl, :], dm, NT)
        dmod[SB_] += _fold(dh2)
        dmod[CB_] += _fold(dh2 * xhat)
        dx1 = gT.astype(f32) + _layernorm_bwd(dh2 * cb, xhat, rstd)
        dx1T[b] = dx1
        dmod[GA_] += _fold(dx1 * attn)
        dattn = (dx1 * ga).astype(bf16)
        do = _dot(wo[...], dattn)
        dwo[...] += _dot(oT, dattn, NT)
        for sl in chunks:
            dw1[sl, :] += _dot(duT[sl, :], h2, NT)

        row = lax.broadcasted_iota(jnp.int32, (8, W), 0)
        for i, win in enumerate(_to_heads(do)):
            o, inv_l = normalized(i)
            dn = _round(win * inv_l)
            prod = dn * o
            part = prod[:8] + prod[8:16] + jnp.where(row < DH - 16, prod[16:], 0.0)
            delta = -jnp.sum(part, axis=0, keepdims=True)
            d0 = _round(delta)
            d1 = _round(delta - d0)
            d2 = _round(delta - d0 - d1)
            tail = jnp.where(row == 4, d0, jnp.where(row == 5, d1, jnp.where(row == 6, d2, dn[16:])))
            OH[i] = jnp.concatenate([dn[:16], tail], axis=0)

    def attention_bwd(b, P, DS0):
        def dscores(h, c, do_w):
            dp = _dot(_unpack(VS[rows(c), :])[:, :32], do_w)
            return (_unpack(P[h, rows(c), :]).astype(f32) * dp).astype(bf16)

        DS0[...] = _pack(dscores(0, 0, _as_weights(OH[0])))

        def body(j, carry):
            ds = _unpack(DS0[...])
            qs = [QH[b * H + BWD_UNROLL * j + i] for i in range(BWD_UNROLL)]
            for i in range(BWD_UNROLL):
                h = BWD_UNROLL * j + i
                do = OH[h]
                do_w = _as_weights(do)
                dq = None
                for c in range(NC):
                    if c + 1 < NC:
                        nxt = dscores(h, c + 1, do_w)
                    else:
                        hn = jnp.minimum(h + 1, H - 1)
                        nxt = dscores(hn, 0, _as_weights(OH[hn]))
                    sl = slice(c * C, (c + 1) * C)
                    DV[:, sl] += _dot(do, _unpack(P[h, rows(c), :]), NT)
                    DK[:, sl] += _dot(qs[i], ds, NT)
                    part = _dot(KT[:, sl], ds)
                    dq = part if dq is None else dq + part
                    ds = nxt
                QH[b * H + h] = dq
            DS0[...] = _pack(ds)
            return carry

        lax.fori_loop(0, H // BWD_UNROLL, body, 0)

    def modulation_bwd(wmod, ks):
        col = _lanes(_column(silu_c), D)
        acc = None
        for k in ks:
            row = _round(jnp.sum(dmod[k].T, axis=0, keepdims=True))
            part = _dot(jnp.broadcast_to(row, (8, D)), wmod[:, k * D:(k + 1) * D], NT)
            acc = part if acc is None else acc + part
            wmod[:, k * D:(k + 1) * D] = (col * row).astype(bf16)
        return acc

    early = [(w1T, dw1T_hbm), (w2, dw2_hbm), (wo, dwo_hbm)]
    early = [pltpu.make_async_copy(s, d, out_sem.at[i]) for i, (s, d) in enumerate(early)]

    def blocks(P):
        def block(b, carry):
            pl.run_scoped(lambda SB, MB: attention_fwd(b, P, SB, MB),
                          pltpu.VMEM((S, W), f32), pltpu.VMEM((8, W), f32))
            pl.run_scoped(lambda aT, duT: dense(b, aT, duT),
                          pltpu.VMEM((F, W), bf16), pltpu.VMEM((F, W), bf16))
            o_copy(b).start()

            @pl.when(b + 1 < NB)
            def _():
                g_copy(b + 1).start()

            @pl.when(b + 1 == NB)
            def _():
                w1T[...] = dw1[...].astype(bf16)
                w2[...] = dw2[...].astype(bf16)
                wo[...] = dwo[...].astype(bf16)
                for cp in early:
                    cp.start()

            pl.run_scoped(lambda DS0: attention_bwd(b, P, DS0), pltpu.VMEM((C // 2, W), u32))
            o_copy(b).wait()
            return carry

        lax.fori_loop(0, NB, block, 0)

    pl.run_scoped(blocks, pltpu.VMEM((H, S // 2, W), u32))

    def epilogue(dxbuf, hT, dqT, wmod):
        lo, hi = pl.ds(0, 2 * D), pl.ds(2 * D, 4 * D)
        fetch = [pltpu.make_async_copy(wmod_hbm.at[:, sl], wmod.at[:, sl], in_sem.at[i])
                 for i, sl in enumerate((hi, lo))]
        for cp in fetch:
            cp.start()
        row = lax.broadcasted_iota(jnp.int32, (HR, S), 0)
        dkv = jnp.concatenate([jnp.where(row < DH, DK[...] * (1.0 / LOG2E), 0.0),
                               jnp.where(row < DH, DV[...], 0.0)], axis=0).astype(bf16)
        wkv_n = wkv[...].T.astype(bf16)[:, :2 * HR]
        ca, sa = _lanes(mod[CA_], W), _lanes(mod[SA_], W)
        late = []
        for b in range(NB):
            sl = slice(b * W, (b + 1) * W)
            dq = (_from_heads([QH[b * H + i] for i in range(H)]) * SCALE).astype(bf16)
            dqT[:, sl] = dq
            dh = _dot(wq[...], dq) + _dot(wkv_n, dkv[:, sl])
            xhat, rstd = _layernorm(_unpack(xT[b]).astype(f32))
            hT[:, sl] = (xhat * ca + sa).astype(bf16)
            dmod[SA_] += _fold(dh)
            dmod[CA_] += _fold(dh * xhat)
            dxbuf[b] = (dx1T[b] + _layernorm_bwd(dh * ca, xhat, rstd)).astype(bf16).T
            late.append(pltpu.make_async_copy(dxbuf.at[b], dx_hbm.at[pl.ds(b * W, W)],
                                              out_sem.at[4 + b]))
            late[-1].start()
            if b == 1:
                fetch[0].wait()
                dsilu = modulation_bwd(wmod, (GA_, SB_, CB_, GB_))
                late.append(pltpu.make_async_copy(wmod.at[:, hi], dwmod_hbm.at[:, hi], out_sem.at[3]))
                late[-1].start()
        fetch[1].wait()
        dsilu = dsilu + modulation_bwd(wmod, (SA_, CA_))
        late.append(pltpu.make_async_copy(wmod.at[:, lo], dwmod_hbm.at[:, lo], out_sem.at[4 + NB]))
        late[-1].start()
        dc_ref[...] = (dsilu[0:1] * (sig_c + cf * sig_c * (1.0 - sig_c))).astype(bf16)
        wq[...] = _dot(hT[...], dqT[...], NT).astype(bf16)
        late.append(pltpu.make_async_copy(wq, dwq_hbm, out_sem.at[5 + NB]))
        late[-1].start()
        dwkv = _dot(dkv, hT[...], NT)
        dwkT_ref[...] = dwkv[0:DH].astype(bf16)
        dwvT_ref[...] = dwkv[HR:HR + DH].astype(bf16)
        for cp in early + late:
            cp.wait()

    pl.run_scoped(epilogue, pltpu.VMEM((NB, W, D), bf16), pltpu.VMEM((D, S), bf16),
                  pltpu.VMEM((D, S), bf16), pltpu.VMEM((D, 6 * D), bf16))


@jax.jit
def pallas_adaLN_cond__grouped_kv_mqa__dense_activation_silu__prompt_kernel(
    A_x: jax.Array,
    A_wq: jax.Array,
    A_wk: jax.Array,
    A_wv: jax.Array,
    A_wo: jax.Array,
    B_x: jax.Array,
    B_w1: jax.Array,
    B_w2: jax.Array,
    c: jax.Array,
    w_mod: jax.Array,
    grad_out: jax.Array,
):
    del B_x
    vmem = pl.BlockSpec(memory_space=pltpu.VMEM)
    hbm = pl.BlockSpec(memory_space=pl.ANY)
    out_shapes = [(S, D), (S, D), (D, D), (DH, D), (DH, D), (D, D), (F, D), (F, D), (1, D), (D, 6 * D)]
    scratch = [
        pltpu.VMEM((NB, D // 2, W), u32),
        pltpu.VMEM((NB * H, HR, W), f32),
        pltpu.VMEM((H, HR, W), f32),
        pltpu.VMEM((S // 2, 128), u32),
        pltpu.VMEM((S // 2, 128), u32),
        pltpu.VMEM((HR, S), f32),
        pltpu.VMEM((HR, S), f32),
        pltpu.VMEM((HR, S), f32),
        pltpu.VMEM((HR, S), f32),
        pltpu.VMEM((D, D), bf16),
        pltpu.VMEM((D, D), bf16),
        pltpu.VMEM((D, D), bf16),
        pltpu.VMEM((F, D), bf16),
        pltpu.VMEM((D, F), bf16),
        pltpu.VMEM((F, D), bf16),
        pltpu.VMEM((D, F), bf16),
        pltpu.VMEM((128, D), f32),
        pltpu.VMEM((F, D), f32),
        pltpu.VMEM((F, D), f32),
        pltpu.VMEM((D, D), f32),
        pltpu.VMEM((NB, D, W), f32),
        pltpu.VMEM((6, D, 128), f32),
        pltpu.VMEM((6, D, 128), f32),
        pltpu.VMEM((W, D), bf16),
        pltpu.VMEM((W, D), bf16),
        pltpu.VMEM((S, W), f32),
        pltpu.VMEM((8, W), f32),
        pltpu.SemaphoreType.DMA((6 + NB,)),
        pltpu.SemaphoreType.DMA(()),
        pltpu.SemaphoreType.DMA(()),
        pltpu.SemaphoreType.DMA((6 + NB,)),
    ]
    out, dx, dwq, dwkT, dwvT, dwo, dw1T, dw2, dc, dwmod = pl.pallas_call(
        _kernel,
        out_shape=[jax.ShapeDtypeStruct(s, bf16) for s in out_shapes],
        in_specs=[vmem] * 3 + [hbm] * 7,
        out_specs=[hbm, hbm, hbm, vmem, vmem, hbm, hbm, hbm, vmem, hbm],
        scratch_shapes=scratch,
        compiler_params=pltpu.CompilerParams(vmem_limit_bytes=127 * 2**20),
        name="adaln_mqa_mlp_fwd_bwd",
    )(c, A_wk.T, A_wv.T, A_x.reshape(S, D), grad_out.reshape(S, D), A_wq, A_wo, B_w1.T, B_w2, w_mod)
    return (out.reshape(1, S, D), dx.reshape(1, S, D), dwq, dwkT.T, dwvT.T, dwo, dw1T.T, dw2, dc, dwmod)
```

```python
import functools
import itertools
import math

import jax
import jax.numpy as jnp
from jax import lax
import jax.experimental.pallas as pl
import jax.experimental.pallas.tpu as pltpu

S, D, H, F = 2048, 640, 32, 1728
DH = D // H
HR = 24
W = 512
NB = S // W
C = 128
NC = S // C
FP = 1792
NV = 16
EARLY, EARLY_PINS = (2, 6, 10, 14), (16,)
FWD_UNROLL, FWD_LAG, FWD_PINS, FWD_SKIP = 4, 2, (2, 4, 6, 7), 2
BWD_UNROLL, BWD_PINS, BWD_SKIP = 4, (1, 4, 7, 14), 4
SAFE_SCORE = 50.0
PR, MC = 32, 64
F1, FE = 128, 320
FC, HE = 192, 160
GC, UC, UA = 144, 96, 480
DQ_EARLY = 384
EPS = 1e-5
LOG2E = math.log2(math.e)
SCALE = DH ** -0.5

bf16, f32, u32 = jnp.bfloat16, jnp.float32, jnp.uint32
NN = (((1,), (0,)), ((), ()))
NT = (((1,), (1,)), ((), ()))


def _dot(a, b, dims=NN):
    return lax.dot_general(a, b, dims, preferred_element_type=f32)


def _strassen(a, b, dims=NN, tick=lambda m: m):
    def add(x, y, sign=1):
        x, y = x.astype(f32), y.astype(f32)
        return (x + y if sign > 0 else x - y).astype(bf16)

    m2 = tick(_dot(add(a(1, 0), a(1, 1)), b(0, 0), dims))
    m4 = tick(_dot(a(1, 1), add(b(1, 0), b(0, 0), -1), dims))
    m3 = tick(_dot(a(0, 0), add(b(0, 1), b(1, 1), -1), dims))
    m5 = tick(_dot(add(a(0, 0), a(0, 1)), b(1, 1), dims))
    m1 = tick(_dot(add(a(0, 0), a(1, 1)), add(b(0, 0), b(1, 1)), dims))
    m7 = tick(_dot(add(a(0, 1), a(1, 1), -1), add(b(1, 0), b(1, 1)), dims))
    m6 = tick(_dot(add(a(1, 0), a(0, 0), -1), add(b(0, 0), b(0, 1)), dims))
    return (jnp.concatenate([m4 - m5 + m1 + m7, m3 + m5], axis=1),
            jnp.concatenate([m2 + m4, m3 - m2 + m1 + m6], axis=1))


def _both(sl, total):
    return sl, slice(sl.start + total // 2, sl.stop + total // 2)


def _project(w, pair, x, **kw):
    k, n = 256, W // 2
    rest = [_dot(w[sl, 2 * k:], x[2 * k:]) for sl in pair]
    out = _strassen(lambda i, j: w[pair[i], j * k:(j + 1) * k],
                    lambda i, j: x[i * k:(i + 1) * k, j * n:(j + 1) * n], **kw)
    return [o + r for o, r in zip(out, rest)]


def _outer(a, pair, y, **kw):
    k, n = W // 2, 256
    out = _strassen(lambda i, j: a[pair[i], j * k:(j + 1) * k],
                    lambda i, j: y[j * n:(j + 1) * n, i * k:(i + 1) * k], NT, **kw)
    return [jnp.concatenate([o, _dot(a[sl, :], y[2 * n:], NT)], axis=1) for o, sl in zip(out, pair)]


def _pack(x):
    x = lax.bitcast_convert_type(x, u32).reshape(-1, 2, 8, x.shape[1])
    return ((x[:, 0] >> 16) | (x[:, 1] & u32(0xFFFF0000))).reshape(-1, x.shape[-1])


def _unpack(w):
    halves = [h.reshape(-1, 1, 8, w.shape[1]) for h in (w << 16, w & u32(0xFFFF0000))]
    return lax.bitcast_convert_type(jnp.concatenate(halves, axis=1).reshape(-1, w.shape[1]), f32)


def _pair_order(x, inverse=False):
    key, pos = (lax.broadcasted_iota(jnp.int32, (128, 128), i) for i in ((1, 0) if inverse else (0, 1)))
    pick = jnp.where(key == (pos & ~15) + ((pos & 15) >> 1) + 8 * (pos & 1), 1.0, 0.0).astype(bf16)
    return jnp.concatenate([_dot(x[:, i:i + 128], pick) for i in range(0, x.shape[1], 128)], axis=1)


def _valu_product(table, rows, init=None):
    acc = init
    for d in range(DH):
        term = table[d].reshape(-1, 8, 128) * rows[d][None]
        acc = term if acc is None else acc + term
    return acc.reshape(-1, 128)


class _Spread:
    def __init__(self, jobs, pins, skip, step):
        self.jobs, self.pins, self.skip = list(jobs), pins, skip
        self.keep = lax.broadcasted_iota(jnp.int32, (8, 128), 0) >= -step

    def __call__(self, x, first):
        out = []
        for i in range(x.shape[0] // 8):
            part = x[8 * i:8 * i + 8]
            if first + i in self.pins:
                self.skip -= 1
                if self.skip < 0 and self.jobs:
                    done = self.jobs.pop(0)()
                    done = done if done.shape[0] == 8 else jnp.maximum(done[:8], done[8:])
                    part = jnp.where(self.keep, part, lax.bitcast_convert_type(done, x.dtype))
            out.append(part)
        return jnp.concatenate(out, axis=0)


class _After:
    def __init__(self, step):
        self.keep = lax.broadcasted_iota(jnp.int32, (8, W), 0) >= -step
        self.last = None

    def mark(self, x):
        self.last = x[-8:, :W]
        return x

    def __call__(self, row, n):
        if self.last is None:
            return row
        return jnp.concatenate([jnp.where(self.keep, row, self.last)] * (n // 8), axis=0)


def _round(x):
    return x.astype(bf16).astype(f32)


def _leading(x):
    return lax.bitcast_convert_type(lax.bitcast_convert_type(x, jnp.int32) & -65536, f32)


def _lanes(col, n):
    return jnp.concatenate([col] * (n // 128), axis=1)


def _fold(x):
    out = x[:, :128]
    for i in range(1, x.shape[1] // 128):
        out = out + x[:, i * 128:(i + 1) * 128]
    return out


def _column(row):
    return jnp.broadcast_to(row, (128, D)).T


def _interleave(*lists):
    order = sorted(((i + 0.5) / len(l), k, i) for k, l in enumerate(lists) for i in range(len(l)))
    for _, k, i in order:
        lists[k][i]()


def _over(fn, stop, step, start=0):
    return [functools.partial(fn, slice(r, min(r + step, stop))) for r in range(start, stop, step)]


def _rowsum(x):
    return jnp.sum(x.reshape(-1, 8, x.shape[1]), axis=0)


def _to_heads(x):
    out = []
    for j in range(x.shape[0] // (2 * DH)):
        r = 2 * DH * j
        out.append(x[r:r + HR])
        out.append(pltpu.roll(x[r + 16:r + 16 + HR], DH, 0))
    return out


def _from_heads(heads):
    low = lax.broadcasted_iota(jnp.int32, (8, W), 0) < 4
    rows = []
    for j in range(len(heads) // 2):
        even, odd = heads[2 * j], pltpu.roll(heads[2 * j + 1], HR - DH, 0)
        rows += [even[:16], jnp.where(low, even[16:], odd[:8]), odd[8:]]
    return jnp.concatenate(rows, axis=0)


def _as_weights(x):
    return jnp.concatenate([x, jnp.zeros((128 - HR, W), f32)], axis=0).astype(bf16)


def _kernel(c_hbm, wkT_hbm, wvT_hbm, x_hbm, g_hbm, wq_hbm, wo_hbm, w1T_hbm, w2_hbm, wmod_hbm,
            out_hbm, dx_hbm, dwq_hbm, dwkT_hbm, dwvT_hbm, dwo_hbm, dw1T_hbm, dw2_hbm, dc_hbm,
            dwmod_hbm,
            gates, xT, hT, gT, dm, stats, sums, QH, OH, DS0, KS, VS, KB, VB, KE, hid, KT, VT, DK, DV,
            wo, woT, w1T, w2, wT, wkv,
            dw1, dw2, dwo, dx1T, mod, dmod, io, norms, dgate, cond, in_sem, g_sem, o_sem, out_sem):
    k_words, v_words = KS, VS
    xT, hT, gT, dm, woT, KS, VS, DS0 = (
        ref.bitcast(bf16) for ref in (xT, hT, gT, dm, woT, KS, VS, DS0))
    SA_, CA_, GA_, SB_, CB_, GB_ = range(6)

    def g_copy(b):
        return pltpu.make_async_copy(g_hbm.at[pl.ds(jnp.minimum(b, NB - 1) * W, W)], io.at[b % 2], g_sem)

    def o_copy(b):
        return pltpu.make_async_copy(io.at[b % 2], out_hbm.at[pl.ds(b * W, W)], o_sem)

    def keys(c):
        return slice(c * C, (c + 1) * C)

    def pairs(c, skip=0):
        return slice((c * C + skip) // 2, (c + 1) * C // 2)

    def early_rows(h, e, n=NV // 2):
        return pl.ds(pl.multiple_of((h * len(EARLY) + e) * (NV // 2), 8), n)

    def head_sum(x):
        row = lax.broadcasted_iota(jnp.int32, (8, W), 0)
        return jnp.sum(x[:8] + x[8:16] + jnp.where(row < DH - 16, x[16:], 0.0), axis=0, keepdims=True)

    def replicated(x, n):
        return [[jnp.broadcast_to(x[d:d + 1, t * 128:(t + 1) * 128], (8, 128)) for d in range(n)]
                for t in range(W // 128)]

    lo, hi = pl.ds(0, 2 * D), pl.ds(2 * D, 4 * D)

    def modulation(wmod, first):
        row = _dot(jnp.broadcast_to(cond[0:1, :], (8, D)), wmod[...])[0:1]
        for i in range(wmod.shape[1] // D):
            part = row[:, i * D:(i + 1) * D]
            gates[first + i:first + i + 1, :] = part
            mod[first + i] = _column(part + 1.0 if first + i in (CA_, CB_) else part)

    def add_sums(i, sl, x):
        sums[i] = sums[i] + _rowsum(x) if sl.start else _rowsum(x)

    def mean(i):
        return jnp.sum(sums[i], axis=0, keepdims=True) * (1.0 / D)

    def modulate(x, st, k, sl, after):
        xhat = x * after(st[0:1, :], x.shape[0]) - st[1:2, :]
        return (xhat * _lanes(mod[k + 1, sl, :], W) + _lanes(mod[k, sl, :], W)).astype(bf16)

    def layernorm(x, st, k, out, after):
        def center():
            st[1:2, :] = mean(0)

        def moment(sl):
            add_sums(1, sl, jnp.square(x(sl) - after(st[1:2, :], sl.stop - sl.start)))

        def finish():
            scale = lax.rsqrt(mean(1) + EPS)
            st[0:1, :] = scale
            st[1:2, :] = st[1:2, :] * scale

        def apply(sl):
            out[sl, :] = modulate(x(sl), st, k, sl, after)

        return [center] + _over(moment, D, 2 * PR) + [finish] + _over(apply, D, PR)

    def layernorm_bwd(dh, x, st, k, emit, after):
        def reduce(sl):
            gain, d = _lanes(mod[k + 1, sl, :], W), dh[sl, :]
            dgain = d * (x(sl) * after(st[0:1, :], PR) - st[1:2, :])
            dmod[0, sl, :] += _fold(d)
            dmod[1, sl, :] += _fold(dgain)
            dh[sl, :] = d * gain
            sums[0] += _rowsum(d * gain)
            sums[1] += _rowsum(dgain * gain)

        def finish():
            scale, m2 = st[0:1, :], mean(1) * st[0:1, :]
            st[2:3, :] = scale * m2
            st[3:4, :] = mean(0) * scale - st[1:2, :] * m2

        def apply(sl):
            emit(sl, dh[sl, :] * after(st[0:1, :], PR) - x(sl) * after(st[2:3, :], PR) - st[3:4, :])

        sums[...] = jnp.zeros(sums.shape, f32)
        return reduce, [finish] + _over(apply, D, PR)

    def gather_dq(b, i):
        first = jnp.maximum(b, 0) * H + 4 * jnp.minimum(i, H // 4 - 1)
        heads = [QH[first + j] for j in range(4)]
        words = pltpu.bitcast((_from_heads(heads) * SCALE).astype(bf16), u32)
        valid = jnp.logical_and(b >= 0, i < H // 4)
        old = pltpu.bitcast(jnp.concatenate([heads[0], heads[1][:16]], axis=0), u32)
        words = pltpu.bitcast(jnp.where(valid, words, old), f32)
        QH[first], QH[first + 1, 0:16, :] = words[:HR], words[HR:]

    def load_dq(b):
        words = [QH[b * H + i + j, 0:HR - 8 * j, :] for i in range(0, H, 4) for j in range(2)]
        return pltpu.bitcast(jnp.concatenate(words, axis=0), bf16)

    def grad_in(src, sl):
        g = src[:, sl].T
        gT[sl, :] = g
        gated = g.astype(f32) * _lanes(mod[GB_, sl, :], W)
        dm[sl, :] = gated.astype(bf16)
        return gated

    small = [pltpu.VMEM((1, D), bf16), pltpu.VMEM((DH, D), bf16), pltpu.VMEM((DH, D), bf16)]
    fetch_hi = pltpu.make_async_copy(wmod_hbm.at[:, hi], wT.at[:, pl.ds(0, 4 * D)], in_sem.at[1])
    wq = wT.at[:, pl.ds(4 * D, D)]
    weights = [pltpu.make_async_copy(src, dst, in_sem.at[2 + i]) for i, (src, dst) in
               enumerate([(wq_hbm, wq), (wo_hbm, wo), (w1T_hbm, w1T), (w2_hbm, w2)])]

    def prologue(xbuf, wmod, wqT, c_ref, wkT_ref, wvT_ref):
        wqT = wqT.bitcast(bf16)

        def x_copy(b):
            return pltpu.make_async_copy(x_hbm.at[pl.ds(b * W, W)], xbuf.at[b], in_sem.at[6 + b])

        first = [pltpu.make_async_copy(wmod_hbm.at[:, lo], wmod, in_sem.at[0])]
        first = [pltpu.make_async_copy(src, dst, in_sem.at[6 + NB + i]) for i, (src, dst) in
                 enumerate([(c_hbm, c_ref), (wkT_hbm, wkT_ref), (wvT_hbm, wvT_ref)])] + [x_copy(0)] + first
        for cp in first:
            cp.start()

        def clear(i, carry):
            dw1[pl.ds(pl.multiple_of(i * (F // 8), 8), F // 8), :] = jnp.zeros((F // 8, D), f32)
            dw2[pl.ds(pl.multiple_of(i * (F // 8), 8), F // 8), :] = jnp.zeros((F // 8, D), f32)
            dwo[pl.ds(pl.multiple_of(i * (D // 8), 8), D // 8), :] = jnp.zeros((D // 8, D), f32)
            dmod[:, pl.ds(pl.multiple_of(i * (D // 8), 8), D // 8), :] = jnp.zeros((2, D // 8, 128), f32)
            return carry

        lax.fori_loop(0, 8, clear, 0)
        for cp in [weights[0]] + [x_copy(b) for b in range(1, NB)]:
            cp.start()
        for ref in (wkv, DK, DV, norms):
            ref[...] = jnp.zeros(ref.shape, f32)

        def normalize(b, after):
            def transpose(sl):
                xt = xbuf[b, :, sl].T
                xT[b, sl, :] = xt
                add_sums(0, sl, xt.astype(f32))

            return _over(transpose, D, 128) + layernorm(
                lambda sl: xT[b, sl, :].astype(f32), stats.at[b], SA_, hT.at[b], after)

        for cp in first[:-1]:
            cp.wait()
        wkv[0:DH, :] = wkT_ref[...].astype(f32)
        wkv[HR:HR + DH, :] = wvT_ref[...].astype(f32)
        cf = c_ref[...].astype(f32)
        sig_c = jax.nn.sigmoid(cf)
        cond[0:1, :] = _round(cf * sig_c)
        cond[1:2, :] = sig_c + cf * sig_c * (1.0 - sig_c)
        pieces = normalize(0, lambda row, n: row)
        _interleave(pieces[:-(D // PR)])
        first[-1].wait()
        weights[0].wait()
        weights[1].start()
        fetch_hi.start()
        g_copy(0).start()
        modulation(wmod, SA_)
        wqT[...] = wq[...].T
        _interleave(pieces[-(D // PR):])

        def replicate(table, t):
            t = t.astype(f32)
            for d in range(DH):
                table[d] = jnp.broadcast_to(t[:, d:d + 1], (NV, 128))

        def project(b, after, others, late=()):
            h = hT[b]
            kv = _round(_dot(wkv[0:2 * HR, :], h))
            row = lax.broadcasted_iota(jnp.int32, (HR, W), 0)
            k = kv[:HR]
            norms[1:2, :] = jnp.maximum(norms[1:2, :], head_sum(k * k))
            v = jnp.where(jnp.logical_and(row >= DH, row < DH + 3), 1.0, kv[HR:])
            tables = []
            for t, stream, table in ((k, KS, KB), (v, VS, VB)):
                t = jnp.concatenate([t, jnp.zeros((128 - HR, W), f32)], 0).T.astype(bf16)
                tables += [functools.partial(replicate, table.at[b * (W // C) + i], t[i * C:i * C + NV])
                           for i in range(W // C)]
                if table is KB:
                    r = EARLY[0] * C + NV
                    tables.append(functools.partial(replicate, KE.at[b], t[r:r + NV]))
                stream[pl.ds(pl.multiple_of(b * W, W), W), :] = t

            def queries(sl):
                heads = _to_heads(after.mark(_round(_dot(wqT[sl, :], h) * (SCALE * LOG2E))))
                for i, win in enumerate(heads):
                    QH[b * H + sl.start // DH + i] = win
                norms[0:1, :] = functools.reduce(jnp.maximum, [head_sum(w * w) for w in heads], norms[0:1, :])

            _interleave(_over(queries, D - 4 * DH, 4 * DH), others, tables[:4])
            KT[:, pl.ds(pl.multiple_of(b * W, W), W)] = k
            VT[:, pl.ds(pl.multiple_of(b * W, W), W)] = _pair_order(v)
            _interleave(_over(queries, D, 4 * DH, D - 4 * DH), tables[4:], late)

        def project_step(b, _):
            x_copy(b + 1).wait()
            after = _After(b)
            project(b, after, normalize(b + 1, after))
            return b + 1

        def first_early(h):
            k = jnp.concatenate([k_words[pl.ds((c * C + NV) // 2, NV // 2), :] for c in EARLY], axis=0)
            s = _dot(pltpu.bitcast(k, bf16), _as_weights(QH[h]))
            hid[pl.ds(h * k.shape[0], k.shape[0]), :] = _pack(jnp.exp2(s))

        def transpose_wo(sl):
            woT[sl, :] = wo[:, sl].T

        last = lax.fori_loop(0, NB - 1, project_step, jnp.int32(0))
        for cp in weights[2:]:
            cp.start()
        weights[1].wait()
        fetch_hi.wait()
        g_copy(0).wait()
        columns = [functools.partial(modulation, wT.at[:, pl.ds((k - GA_) * D, D)], k)
                   for k in (GB_, GA_, SB_, CB_)]
        project(last, _After(last), columns + _over(functools.partial(grad_in, io.at[0]), D, 128)
                + _over(transpose_wo, D, 128), [functools.partial(first_early, h) for h in range(H)])

    pl.run_scoped(prologue, pltpu.VMEM((NB, W, D), bf16), pltpu.VMEM((D, 2 * D), bf16),
                  pltpu.VMEM((D // 2, D), u32), *small)

    bounded = jnp.max(norms[0:1, :]) * jnp.max(norms[1:2, :]) <= SAFE_SCORE ** 2

    def attention_fwd(b, P):
        def bounded_heads(i, carry):
            heads = [i * FWD_UNROLL + j for j in range(FWD_UNROLL)]
            q_rows = [replicated(QH[b * H + h], DH) for h in heads]
            words, queue = {}, []

            def job(j, c, t):
                if (j, c, t) not in words:
                    words[j, c, t] = _pack(jnp.exp2(_valu_product(KB.at[c], q_rows[j][t])))
                    P[heads[j], pl.ds(c * C // 2, NV // 2), t * 128:(t + 1) * 128] = words[j, c, t]
                return words[j, c, t]

            def values(j, c):
                for t in range(W // 128):
                    job(j, c, t)
                o = _dot(VT[:, keys(c)], pltpu.bitcast(P[heads[j], pairs(c), :], bf16))
                OH[heads[j]] = OH[heads[j]] + o if c else o

            spread = _Spread([functools.partial(job, j, c, t) for j in range(FWD_UNROLL)
                              for c in range(NC) for t in range(W // 128)], FWD_PINS, FWD_SKIP, i)
            for j, h in enumerate(heads):
                q = _as_weights(QH[b * H + h])
                for c in range(NC):
                    n = 2 * NV if c in EARLY else NV
                    if c in EARLY:
                        P[h, pl.ds((c * C + NV) // 2, NV // 2), :] = hid[early_rows(h, EARLY.index(c)), :]
                    s = _dot(pltpu.bitcast(spread(k_words[pairs(c, n), :], n // NV), bf16), q)
                    P[h, pairs(c, n), :] = _pack(jnp.exp2(s))
                    queue.append(functools.partial(values, j, c))
                    if len(queue) > FWD_LAG:
                        queue.pop(0)()
            for rest in queue:
                rest()
            return carry

        def general_head(h, carry):
            q, n = _as_weights(QH[b * H + h]), 4 * C

            def row_max(i, m):
                s = _dot(KS[pl.ds(pl.multiple_of(i * n, n), n), :], q)
                return jnp.maximum(m, jnp.max(s, axis=0, keepdims=True))

            def values(i, o):
                sl = pl.ds(pl.multiple_of(i * n, n), n)
                p = _pack(jnp.exp2(_dot(KS[sl, :], q) - m))
                P[h, pl.ds(pl.multiple_of(i * (n // 2), n // 2), n // 2), :] = p
                return o + _dot(VT[:, sl], pltpu.bitcast(p, bf16))

            m = lax.fori_loop(0, S // n, row_max, jnp.full((1, W), -jnp.inf, f32))
            OH[h] = lax.fori_loop(0, S // n, values, jnp.zeros((HR, W), f32))
            return carry

        @pl.when(jnp.logical_not(bounded))
        def _():
            lax.fori_loop(0, H, general_head, 0)

        @pl.when(bounded)
        def _():
            lax.fori_loop(0, H // FWD_UNROLL, bounded_heads, 0)

    def dense(b, P, dah, *packed):
        h2, oT = (ref.bitcast(bf16) for ref in packed)
        aT, duT = hid.bitcast(bf16).at[0:FP], hid.bitcast(bf16).at[FP:2 * FP]
        dx1, dattn = aT.at[0:D], aT.at[D:2 * D]
        gbuf, gnext = io.at[b % 2], io.at[(b + 1) % 2]

        row = lax.broadcasted_iota(jnp.int32, (8, W), 0)

        def normalized(i):
            raw = OH[i]
            inv = jnp.broadcast_to(1.0 / after(raw[DH:DH + 1], 8), (8, W))
            o = [raw[:8] * inv, raw[8:16] * inv, jnp.where(row < DH - 16, raw[16:] * inv, inv)]
            o = OH[i] = jnp.concatenate(o, axis=0)
            return o

        g_copy(b + 1).wait()
        x1, st, after = dx1T.at[b], stats.at[NB], _After(b)

        def attend(o, sl):
            for sl, attn in zip(_both(sl, D), _project(woT, _both(sl, D), o)):
                x = xT[b, sl, :].astype(f32) + _lanes(mod[GA_, sl, :], W) * attn
                x1[sl, :] = x
                add_sums(0, sl, x)

        def gather(sl):
            heads = [normalized(i) for i in range(sl.start // DH, sl.stop // DH)]
            oT[sl, :] = _from_heads(heads).astype(bf16)

        def paced(jobs, ticks):
            count = itertools.count()

            def tick(m):
                after.mark(_lanes(m[:, :128], W))
                i = next(count)
                _interleave(jobs[i * len(jobs) // ticks:(i + 1) * len(jobs) // ticks])
                return m

            return tick

        def ahead(g, sl, tick=None):
            pair = _both(sl, F)
            da = _project(w2, pair, g, tick=tick) if tick else [_dot(w2[r, :], g) for r in pair]
            for sl, da in zip(_both(sl, 2 * FE), da):
                dah[sl, :] = after.mark(da)

        def hidden(g, h, sl):
            pair = _both(sl, F)
            da = [dah[r, :] for r in _both(sl, 2 * FE)] if sl.stop <= FE else _project(w2, pair, g)
            for sl, da, u in zip(pair, da, _project(w1T, pair, h)):
                sig = 0.5 * jnp.tanh(0.5 * u) + 0.5
                a = u * sig
                aT[sl, :] = a.astype(bf16)
                duT[sl, :] = (da * (sig + a * (1.0 - sig))).astype(bf16)

        def accumulate(acc, w, sl, update, k=None):
            raw = after.mark(acc[sl, :] + update)
            acc[sl, :] = raw
            old = w[sl, :]
            if k is not None:
                part = _rowsum(raw * old.astype(f32))
                dgate[k // 3] = dgate[k // 3] + part if sl.start else part
                raw = raw * gates[k:k + 1, :]
            w[sl, :] = jnp.where(b + 1 == NB, raw.astype(bf16), old)

        def transpose(sl):
            for col, w in ((0, w2), (FP, w1T)):
                pad = [jnp.zeros((FP - F, D), bf16)] if sl.stop == F else []
                t = jnp.concatenate([w[sl, :]] + pad, axis=0).T
                wT[:, col + sl.start:col + sl.start + t.shape[1]] = t

        def weight_grad(acc, w, a, y, k, sl, **kw):
            pair = _both(sl, w.shape[0])
            for sl, update in zip(pair, _outer(a, pair, y, **kw)):
                accumulate(acc, w, sl, update, k)

        uses = itertools.count(NB)

        def fresh(start, size):
            return pl.ds(pl.multiple_of(start + 16 * jnp.maximum(b - next(uses), 0), 16), size)

        def down(col, x, jobs):
            m, k, n = D // 2, FP // 2, W // 2
            return jnp.concatenate(_strassen(
                lambda i, j: wT[fresh(i * m, m), col + j * k:col + (j + 1) * k],
                lambda i, j: x[fresh(i * k, k), j * n:(j + 1) * n], tick=paced(jobs, 5)), axis=0)

        def output(mlp, sl):
            gbuf[:, sl] = (x1[sl, :] + _lanes(mod[GB_, sl, :], W) * mlp[sl]).astype(bf16).T

        def emit(sl, dx):
            dx = gT[sl, :].astype(f32) + dx
            x1[sl, :] = dx
            dx1[sl, :] = dx.astype(bf16)
            dattn[sl, :] = (dx * _lanes(mod[GA_, sl, :], W)).astype(bf16)

        def out_grad(d, sl):
            for sl, do in zip(_both(sl, D), _project(wo, _both(sl, D), d)):
                dah[sl, :] = after.mark(do)

        def head_grads(sl):
            for i, win in enumerate(_to_heads(dah[sl, :]), sl.start // DH):
                o = OH[i]
                dn = _round(win * after(o[DH:DH + 1], HR))
                delta = -head_sum(dn * o)
                d0 = _leading(delta)
                d1 = _leading(delta - d0)
                d2 = delta - d0 - d1
                tail = jnp.where(row == 4, d0, jnp.where(row == 5, d1, jnp.where(row == 6, d2, dn[16:])))
                OH[i] = jnp.concatenate([dn[:16], jnp.where(row == 7, delta, tail)], axis=0)

        part, g = functools.partial, dm[...]
        _interleave(_over(part(ahead, g), F1, MC), _over(gather, D, 4 * DH))
        attend(oT[...], slice(0, D // 2))
        tick = paced(layernorm(lambda sl: x1[sl, :], st, SB_, h2, after), 7 * ((FE - F1) // MC))
        _interleave(_over(part(ahead, g, tick=tick), FE, MC, F1))
        h = h2[...]
        _interleave(_over(part(hidden, g, h), F // 2, FC, FE), _over(part(hidden, g, h), FE, HE),
                    _over(transpose, F, 256))
        down_grad = part(weight_grad, dw2, w2, aT, gT[...], GB_)
        _interleave(_over(down_grad, F // 2, GC))
        reduce, apply = layernorm_bwd(dah, lambda sl: x1[sl, :], st, SB_, emit, after)
        for x in (aT, duT):
            x[F:FP, :] = jnp.zeros((FP - F, W), bf16)
        dah[...] = down(FP, duT, [part(gather_dq, b - 1, i) for i in range(H // 4)])
        _interleave(_over(part(output, down(0, aT, _over(reduce, D, PR))), D, 128))
        up_grad = part(weight_grad, dw1, w1T, duT, h, None)
        _interleave(_over(part(up_grad, tick=paced(apply, 7 * (UA // UC))), UA, UC))
        up_grad(slice(UA, UA + UC))
        out_grad(dattn[...], slice(0, D // 2))
        tick = paced(_over(lambda sl: after.mark(grad_in(gnext, sl)), D, 128) + _over(head_grads, D, 2 * DH),
                     7 * (D // 2 // 80 + (F // 2 - UA) // UC - 2))
        _interleave(_over(part(weight_grad, dwo, wo, oT, dx1[...], GA_, tick=tick), D // 2, 80)
                    + _over(part(up_grad, tick=tick), F // 2 - UC, UC, UA + UC))
        DS0[...] = dscores(P, 0, 0, 0, VS[keys(0), :], _as_weights(OH[0])).astype(bf16)
        up_grad(slice(F // 2 - UC, F // 2))

    def dscores(P, h, c, n, v, do_w):
        return _unpack(P[h, pairs(c, n), :]) * _dot(v, do_w)

    def attention_bwd(b, P):
        def body(i, carry):
            heads = [i * BWD_UNROLL + j for j in range(BWD_UNROLL)]
            heads.append(jnp.minimum(heads[-1] + 1, H - 1))
            do_rows = [replicated(OH[h], HR) for h in heads[:-1]]
            words = {}

            def valu(j, c):
                return NV if c or j % BWD_UNROLL else 0

            def job(j, c, t):
                if (j, c, t) not in words:
                    dp = _valu_product(VB.at[c], do_rows[j][t], do_rows[j][t][HR - 1][None])
                    p = P[heads[j], pl.ds(c * C // 2, NV // 2), t * 128:(t + 1) * 128]
                    words[j, c, t] = _unpack(p) * dp
                return words[j, c, t]

            spread = _Spread([functools.partial(job, j, c, t) for j in range(BWD_UNROLL)
                              for c in range(NC) if valu(j, c) for t in range(W // 128)],
                             BWD_PINS, BWD_SKIP, i)
            q_rows = [replicated(QH[jnp.where(b + 1 < NB, b + 1, b) * H + h], DH) for h in heads[:-1]]

            def early_job(j, e, t):
                w = _pack(jnp.exp2(_valu_product(KE.at[e], q_rows[j][t])))
                hid[early_rows(heads[j], e), t * 128:(t + 1) * 128] = w
                return w

            extra = _Spread([functools.partial(early_job, j, e, t) for j in range(BWD_UNROLL)
                             for t in range(W // 128) for e in range(len(EARLY))], EARLY_PINS, 0, i)
            nxt, do_w = DS0[...], _as_weights(OH[heads[0]])
            for j, h in enumerate(heads[:-1]):
                dq = None
                for c in range(NC):
                    if valu(j, c):
                        first = jnp.concatenate([job(j, c, t) for t in range(W // 128)], axis=1)
                        nxt = jnp.concatenate([first, nxt], axis=0)
                    ds = nxt.astype(bf16)
                    j1, c1 = j + (c + 1) // NC, (c + 1) % NC
                    n = valu(j1, c1)
                    if c1 == 0:
                        do_w = _as_weights(OH[heads[j1]])
                    v = spread(v_words[pairs(c1, n), :], n // 16)
                    nxt = dscores(P, heads[j1], c1, n, pltpu.bitcast(v, bf16), do_w)
                    sl = keys(c)
                    DV[:, sl] += _dot(OH[h], pltpu.bitcast(P[h, pairs(c), :], bf16), NT)
                    DK[:, sl] += _dot(QH[b * H + h], ds, NT)
                    part = _dot(extra(spread(KT[:, sl], 14), 14), ds)
                    dq = part if dq is None else dq + part
                QH[b * H + h] = dq
            assert not extra.jobs
            DS0[...] = nxt.astype(bf16)
            return carry

        lax.fori_loop(0, H // BWD_UNROLL, body, 0)

    early = [pltpu.make_async_copy(src, dst, out_sem.at[4 + i]) for i, (src, dst) in
             enumerate([(w1T, dw1T_hbm), (w2, dw2_hbm), (wo, dwo_hbm)])]

    def reduce_dmod(k):
        for i in range(2):
            gates[k + i:k + i + 1, :] = jnp.sum(dmod[i].T, axis=0, keepdims=True)

    def block(b, P):
        g_copy(b + 1).start()
        pl.run_scoped(functools.partial(attention_fwd, b, P))

        @pl.when(b == 0)
        def _():
            for cp in weights[2:]:
                cp.wait()

        pl.run_scoped(functools.partial(dense, b, P), pltpu.VMEM((D, W), f32),
                      *[pltpu.VMEM((D // 2, W), u32)] * 2)
        o_copy(b).start()

        @pl.when(b + 1 == NB)
        def _():
            for cp in [fetch_hi, weights[0]] + early:
                cp.start()

        pl.run_scoped(functools.partial(attention_bwd, b, P))
        o_copy(b).wait()

    def epilogue(dxbuf, dkv, wkv_n, dwkv, dwq, wmod, silu_c, dh, dxT,
                 dc_ref, dwkT_ref, dwvT_ref):
        dxT = dxT.bitcast(bf16)

        def stores(b):
            col = pl.multiple_of(b * D, 128)
            pairs = [(dxbuf.at[b], dx_hbm.at[pl.ds(b * W, W)]),
                     (wT.at[:, pl.ds(col, D)], dwmod_hbm.at[:, pl.ds(col + 2 * D, D)])]
            return [pltpu.make_async_copy(src, dst, out_sem.at[7 + 2 * b + i])
                    for i, (src, dst) in enumerate(pairs)]

        def modulation_bwd(k, w_ref, col):
            def piece(sl):
                row = _round(gates[pl.ds(k, 1), :])
                cond[2:3, sl] += _dot(jnp.broadcast_to(row, (8, D)), w_ref[sl, pl.ds(col, D)], NT)[0:1]
                w_ref[sl, pl.ds(col, D)] = (_lanes(silu_c[sl, :], D) * row).astype(bf16)

            return _over(piece, D, 128)

        fetch = pltpu.make_async_copy(wmod_hbm.at[:, lo], wmod, in_sem.at[0])
        fetch.start()
        fetch_hi.wait()
        weights[0].wait()
        silu_c[...] = _column(cond[0:1, :])
        row = lax.broadcasted_iota(jnp.int32, (HR, S), 0)
        dkv[...] = jnp.concatenate([jnp.where(row < DH, DK[...] * (1.0 / LOG2E), 0.0),
                                    jnp.where(row < DH, _pair_order(_round(DV[...]), True), 0.0)], axis=0).astype(bf16)
        wkv_n[...] = jnp.concatenate([wkv[...], jnp.zeros((64, D), f32)], axis=0).T.astype(bf16)
        dwkv[...] = jnp.zeros(dwkv.shape, f32)
        reduce_dmod(SB_)
        for k in (GA_, GB_):
            gates[k:k + 1, :] = jnp.sum(dgate[k // 3], axis=0, keepdims=True)
        dmod[...] = jnp.zeros(dmod.shape, f32)
        cond[2:3, :] = jnp.zeros((1, D), f32)

        def body(b, carry):
            after = _After(b)
            dq, dkv_b = load_dq(b), dkv[:, pl.ds(pl.multiple_of(b * W, W), W)]

            def x(sl):
                return xT[b, sl, :].astype(f32)

            def input_grad(sl):
                dh[sl, :] = _dot(wq[sl, :], dq) + _dot(wkv_n[sl, :2 * HR], dkv_b)
                _interleave(_over(reduce, sl.stop, PR, sl.start))

            def emit(sl, dx):
                dxT[sl, :] = (dx1T[b, sl, :] + dx).astype(bf16)
                if sl.stop % 128 == 0:
                    dxbuf[b, :, sl.stop - 128:sl.stop] = dxT[sl.stop - 128:sl.stop, :].T

            def query_grad(sl):
                dwo[sl, :] = after.mark(jnp.where(b > 0, dwo[sl, :], 0.0) + _dot(hT[b, sl, :], dq, NT))

            def kv_grad():
                dwkv[...] += _dot(dkv_b, hT[b], NT)

            reduce, apply = layernorm_bwd(dh, x, stats.at[b], SA_, emit, after)
            _interleave(_over(input_grad, D, MC), modulation_bwd(GA_ + b, wT, pl.multiple_of(b * D, 128)))
            _interleave(_over(query_grad, DQ_EARLY, 64) + [kv_grad], apply,
                        [functools.partial(gather_dq, NB - 1, 3 * b + i) for i in range(3)])
            for cp in stores(b):
                cp.start()
            return carry

        lax.fori_loop(0, NB, body, 0)
        fetch.wait()
        reduce_dmod(SA_)

        def remaining(sl):
            dwq[sl, :] = sum(_dot(hT[b, sl, :], load_dq(b), NT) for b in range(NB)).astype(bf16)

        mid = (DQ_EARLY + D) // 2
        top, rest = pl.ds(0, mid), pl.ds(mid, D - mid)
        dwq[0:DQ_EARLY, :] = dwo[0:DQ_EARLY, :].astype(bf16)
        _interleave(_over(remaining, mid, 64, DQ_EARLY),
                    modulation_bwd(SA_, wmod, 0) + modulation_bwd(CA_, wmod, D))
        late = [pltpu.make_async_copy(wmod, dwmod_hbm.at[:, lo], out_sem.at[1])]
        late[-1].start()
        dc_ref[...] = (cond[2:3, :] * cond[1:2, :]).astype(bf16)
        dwkT_ref[...] = dwkv[0:DH, :].astype(bf16)
        dwvT_ref[...] = dwkv[HR:HR + DH, :].astype(bf16)
        for i, pair in enumerate([(dc_ref, dc_hbm), (dwkT_ref, dwkT_hbm), (dwvT_ref, dwvT_hbm)]):
            late.append(pltpu.make_async_copy(*pair, in_sem.at[6 + NB + i]))
            late[-1].start()
        late.append(pltpu.make_async_copy(dwq.at[top], dwq_hbm.at[top], out_sem.at[2]))
        late[-1].start()
        remaining(rest)
        late.append(pltpu.make_async_copy(dwq.at[rest], dwq_hbm.at[rest], out_sem.at[3]))
        late[-1].start()
        for cp in early + [cp for b in range(NB) for cp in stores(b)] + late:
            cp.wait()

    def step(b, carry):
        pl.run_scoped(functools.partial(block, b), pltpu.VMEM((H, S // 2, W), u32))

        @pl.when(b + 1 == NB)
        def _():
            pl.run_scoped(epilogue, pltpu.VMEM((NB, W, D), bf16), pltpu.VMEM((2 * HR, S), bf16),
                          pltpu.VMEM((D, 128), bf16), pltpu.VMEM((2 * HR, D), f32),
                          pltpu.VMEM((D, D), bf16), pltpu.VMEM((D, 2 * D), bf16),
                          pltpu.VMEM((D, 128), f32), pltpu.VMEM((D, W), f32),
                          pltpu.VMEM((D // 2, W), u32), *small)

        return carry

    lax.fori_loop(0, NB, step, 0)


@jax.jit
def pallas_adaLN_cond__grouped_kv_mqa__dense_activation_silu__prompt_kernel(
    A_x: jax.Array,
    A_wq: jax.Array,
    A_wk: jax.Array,
    A_wv: jax.Array,
    A_wo: jax.Array,
    B_x: jax.Array,
    B_w1: jax.Array,
    B_w2: jax.Array,
    c: jax.Array,
    w_mod: jax.Array,
    grad_out: jax.Array,
):
    del B_x
    hbm = pl.BlockSpec(memory_space=pl.ANY)
    out_shapes = [(S, D), (S, D), (D, D), (DH, D), (DH, D), (D, D), (F, D), (F, D), (1, D), (D, 6 * D)]
    scratch = [
        pltpu.VMEM((24, D), f32),
        pltpu.VMEM((NB, D // 2, W), u32),
        pltpu.VMEM((NB, D // 2, W), u32),
        pltpu.VMEM((D // 2, W), u32),
        pltpu.VMEM((D // 2, W), u32),
        pltpu.VMEM((NB + 1, 8, W), f32),
        pltpu.VMEM((2, 8, W), f32),
        pltpu.VMEM((NB * H, HR, W), f32),
        pltpu.VMEM((H, HR, W), f32),
        pltpu.VMEM((C // 2, W), u32),
        pltpu.VMEM((S // 2, 128), u32),
        pltpu.VMEM((S // 2, 128), u32),
        pltpu.VMEM((NC, DH, NV, 128), f32),
        pltpu.VMEM((NC, DH, NV, 128), f32),
        pltpu.VMEM((len(EARLY), DH, NV, 128), f32),
        pltpu.VMEM((FP, W), u32),
        pltpu.VMEM((HR, S), f32),
        pltpu.VMEM((HR, S), f32),
        pltpu.VMEM((HR, S), f32),
        pltpu.VMEM((HR, S), f32),
        pltpu.VMEM((D, D), bf16),
        pltpu.VMEM((D // 2, D), u32),
        pltpu.VMEM((F, D), bf16),
        pltpu.VMEM((F, D), bf16),
        pltpu.VMEM((D, 2 * FP), bf16),
        pltpu.VMEM((64, D), f32),
        pltpu.VMEM((F, D), f32),
        pltpu.VMEM((F, D), f32),
        pltpu.VMEM((D, D), f32),
        pltpu.VMEM((NB, D, W), f32),
        pltpu.VMEM((6, D, 128), f32),
        pltpu.VMEM((2, D, 128), f32),
        pltpu.VMEM((2, W, D), bf16),
        pltpu.VMEM((8, W), f32),
        pltpu.VMEM((4, 8, D), f32),
        pltpu.VMEM((16, D), f32),
        pltpu.SemaphoreType.DMA((9 + NB,)),
        pltpu.SemaphoreType.DMA(()),
        pltpu.SemaphoreType.DMA(()),
        pltpu.SemaphoreType.DMA((7 + 2 * NB,)),
    ]
    out, dx, dwq, dwkT, dwvT, dwo, dw1T, dw2, dc, dwmod = pl.pallas_call(
        _kernel,
        out_shape=[jax.ShapeDtypeStruct(s, bf16) for s in out_shapes],
        in_specs=[hbm] * 10,
        out_specs=[hbm] * 10,
        scratch_shapes=scratch,
        compiler_params=pltpu.CompilerParams(vmem_limit_bytes=128 * 2**20),
        name="adaln_mqa_mlp_fwd_bwd",
    )(c, A_wk.T, A_wv.T, A_x.reshape(S, D), grad_out.reshape(S, D), A_wq, A_wo, B_w1.T, B_w2, w_mod)
    return (out.reshape(1, S, D), dx.reshape(1, S, D), dwq, dwkT.T, dwvT.T, dwo, dw1T.T, dw2, dc, dwmod)
```
